```python
import os as _os
_os.environ.setdefault("JAX_PLATFORMS", "cpu")
import jax
import jax.numpy as jnp

def _softmax(x, axis=-1):
    return jax.nn.softmax(x, axis=axis)
def _gelu(x):
    return jax.nn.gelu(x, approximate=True)
def _silu(x):
    return jax.nn.silu(x)
def _sigmoid(x):
    return jax.nn.sigmoid(x)
def _layernorm(x, axis=-1, eps=1e-5):
    m = jnp.mean(x, axis=axis, keepdims=True)
    v = jnp.var(x, axis=axis, keepdims=True)
    return (x - m) / jnp.sqrt(v + eps)
def _scatter_add(tgt, idx, src, axis=0):
    return tgt.at[idx].add(src)
def _segment_sum(src, seg, n):
    return jax.ops.segment_sum(src, seg, n)
class _Rng:
    def __init__(self, key):
        self._k = key
    def _next(self):
        self._k, sub = jax.random.split(self._k)
        return sub
    def normal(self, shape):
        return jax.random.normal(self._next(), shape, dtype=jnp.bfloat16)
    def randint(self, lo, hi, shape):
        return jax.random.randint(self._next(), shape, lo, hi, dtype=jnp.int32)
    def uniform(self, shape, lo=0.0, hi=1.0):
        return jax.random.uniform(self._next(), shape, jnp.bfloat16, lo, hi)
    def permutation(self, n):
        return jax.random.permutation(self._next(), n)


kernel_name = 'standalone__gqa_block_cached__near_ridge'

def setup_inputs():
    _rng = _Rng(jax.random.key(int.from_bytes(__import__("os").urandom(4), "little")))
    _w = (lambda a: (lambda t: t.astype(jnp.bfloat16) if jnp.issubdtype(t.dtype, jnp.floating) else t)(jnp.asarray(a)))
    B, Sq, D = 32, 112, 448
    Hq, Hkv, Sk, Dh = 16, 8, 512, 256
    assert Hq % Hkv == 0, (Hq, Hkv)
    return {
        "x": _w((lambda *s: _rng.normal(s) * 0.8)(B, Sq, D)),
        "k_cache": _w((lambda *s: _rng.normal(s) * 0.8)(B, Hkv, Sk, Dh)),
        "v_cache": _w((lambda *s: _rng.normal(s) * 0.05)(B, Hkv, Sk, Dh)),
        "wq": _w((lambda *s: _rng.normal(s) * 0.8)(D, Hq * Dh) * (D ** -0.5)),
        "wo": _w((lambda *s: _rng.normal(s) * 0.05)(Hq * Dh, D) * ((Hq * Dh) ** -0.5)),
    }

def reference(x, k_cache, v_cache, wq, wo):
    B, Sq, D = x.shape
    Hq, Dh = 16, 256
    Hkv = k_cache.shape[1]
    rep = Hq // Hkv
    q = (lambda x, *d: x.transpose(*d))((x @ wq).reshape(B, Sq, Hq, Dh), 0, 2, 1, 3)
    k = jnp.repeat(k_cache, rep, axis=1)
    v = jnp.repeat(v_cache, rep, axis=1)
    scores = jnp.einsum("bhqd,bhkd->bhqk", q, k) * (Dh ** -0.5)
    p = _softmax(scores, axis=-1)
    o = jnp.einsum("bhqk,bhkd->bhqd", p, v)
    return (lambda x, *d: x.transpose(*d))(o, 0, 2, 1, 3).reshape(B, Sq, Hq * Dh) @ wo
```

```python
import jax
import jax.numpy as jnp
from jax import lax
import jax.experimental.pallas as pl
import jax.experimental.pallas.tpu as pltpu

NB = 2
GS = 4
LOG2E = 1.4426950408889634
NT = (((1,), (1,)), ((), ()))
NSLOT = 4

@jax.jit
def pallas_standalone__gqa_block_cached__near_ridge_kernel(x, k_cache, v_cache, wq, wo):
    B, Sq, D = x.shape
    _, Hkv, Sk, Dh = k_cache.shape
    HD = wq.shape[1]
    Hq = HD // Dh
    rep = Hq // Hkv
    GW = rep * Dh
    c = LOG2E * (Dh ** -0.5)
    x2 = x.reshape(B * Sq, D)
    woT = wo.T
    wq3 = wq
    M = NB * Sq
    nsteps = B // NB
    T = GS * M
    ngroups = nsteps // GS
    f32, bf16 = jnp.float32, jnp.bfloat16
    S_X = 0
    S_WQ = S_X + ngroups
    S_WO = S_WQ + Hkv
    S_KV = S_WO + 1
    NSEM = S_KV + NSLOT

    def kernel(x_hbm, k_hbm, v_hbm, wq_hbm, wo_hbm, o_ref,
               x_buf, wq_buf, wo_buf, k_buf, v_buf, q_scr, a_scr, sems):
        i = pl.program_id(0)
        slot = i % NSLOT

        def x_copy(j):
            return pltpu.make_async_copy(x_hbm.at[j * T:(j + 1) * T], x_buf.at[j * T:(j + 1) * T],
                                         sems.at[S_X + j])

        def wq_copy(g):
            return pltpu.make_async_copy(wq_hbm.at[:, pl.ds(g * GW, GW)],
                                         wq_buf.at[g], sems.at[S_WQ + g])

        def wo_copy():
            return pltpu.make_async_copy(wo_hbm, wo_buf, sems.at[S_WO])

        def kv_copies(step, sl):
            return [
                pltpu.make_async_copy(k_hbm.at[pl.ds(step * NB, NB)], k_buf.at[sl], sems.at[S_KV + sl]),
                pltpu.make_async_copy(v_hbm.at[pl.ds(step * NB, NB)], v_buf.at[sl], sems.at[S_KV + sl]),
            ]

        def qproj(xrow0, g):
            xb = x_buf[pl.ds(xrow0, T), :]
            q = jnp.dot(xb, wq_buf[g], preferred_element_type=f32)
            q_scr[g] = q.astype(bf16)

        @pl.when(i == 0)
        def _():
            x_copy(0).start()
            for g in range(Hkv):
                wq_copy(g).start()
            for st in range(NSLOT - 1):
                for cp in kv_copies(st, st):
                    cp.start()
            x_copy(0).wait()

            def qloop(g, carry):
                pltpu.make_async_copy(wq_hbm.at[:, pl.ds(0, GW)], wq_buf.at[g], sems.at[S_WQ + g]).wait()
                qproj(0, g)
                return carry
            lax.fori_loop(0, Hkv, qloop, 0)

        @pl.when(i + NSLOT - 1 < nsteps)
        def _():
            nxt = i + NSLOT - 1
            for cp in kv_copies(nxt, nxt % NSLOT):
                cp.start()

        @pl.when(i == 0)
        def _():
            x_copy(1).start()
            wo_copy().start()

        @pl.when(i == 2)
        def _():
            for j in range(2, ngroups):
                x_copy(j).start()

        for j in range(1, ngroups):
            @pl.when(i == GS * j)
            def _():
                x_copy(j).wait()

        @pl.when(jnp.logical_and(i % GS == 0, i > 0))
        def _():
            xrow = pl.multiple_of(i * M, 16)
            for g in range(Hkv):
                qproj(xrow, g)

        rloc = pl.multiple_of((i % GS) * M, 16)

        def qk(b, g):
            qs = jnp.concatenate(
                [q_scr[g, pl.ds(rloc + b * Sq, Sq), j * Dh:(j + 1) * Dh] for j in range(rep)], axis=0)
            return lax.dot_general(qs, k_buf[slot, b, g], NT, preferred_element_type=f32)

        def pv(b, g, s):
            c0 = g * GW
            m = jnp.max(s, axis=-1, keepdims=True)
            p = jnp.exp2((s - m) * c)
            l = jnp.sum(p, axis=-1, keepdims=True)
            p = p * (1.0 / l)
            o = jnp.dot(p.astype(bf16), v_buf[slot, b, g], preferred_element_type=f32).astype(bf16)
            for j in range(rep):
                a_scr[pl.ds(rloc + b * Sq, Sq), c0 + j * Dh:c0 + (j + 1) * Dh] = o[j * Sq:(j + 1) * Sq]

        items = [(b, g) for g in range(Hkv) for b in range(NB)]
        for cp in kv_copies(i, slot):
            cp.wait()
        s = qk(*items[0])
        for n, it in enumerate(items):
            s_next = qk(*items[n + 1]) if n + 1 < len(items) else None
            pv(*it, s)
            s = s_next

        @pl.when(i == GS - 1)
        def _():
            wo_copy().wait()

        @pl.when(i % GS == GS - 1)
        def _():
            for n in range(T // 128):
                r = lax.dot_general(wo_buf[...], a_scr[n * 128:(n + 1) * 128, :], NT,
                                    preferred_element_type=f32)
                o_ref[n * 128:(n + 1) * 128, :] = r.T.astype(o_ref.dtype)

    any_spec = pl.BlockSpec(memory_space=pl.ANY)
    out = pl.pallas_call(
        kernel,
        grid=(nsteps,),
        in_specs=[any_spec] * 5,
        out_specs=pl.BlockSpec((T, D), lambda i: (i // GS, 0)),
        out_shape=jax.ShapeDtypeStruct((B * Sq, D), x.dtype),
        scratch_shapes=[
            pltpu.VMEM((B * Sq, D), bf16),
            pltpu.VMEM((Hkv, D, GW), bf16),
            pltpu.VMEM((D, HD), bf16),
            pltpu.VMEM((NSLOT, NB, Hkv, Sk, Dh), bf16),
            pltpu.VMEM((NSLOT, NB, Hkv, Sk, Dh), bf16),
            pltpu.VMEM((Hkv, T, GW), bf16),
            pltpu.VMEM((T, HD), bf16),
            pltpu.SemaphoreType.DMA((NSEM,)),
        ],
        compiler_params=pltpu.CompilerParams(
            dimension_semantics=("arbitrary",), vmem_limit_bytes=110 * 1024 * 1024),
    )(x2, k_cache, v_cache, wq3, woT)
    return out.reshape(B, Sq, D)
```

```python
import jax
import jax.numpy as jnp
from jax import lax
import jax.experimental.pallas as pl
import jax.experimental.pallas.tpu as pltpu

NB = 4
GB = 8
NSLOT = 3
QH = 2
LOG2E = 1.4426950408889634
NT = (((1,), (1,)), ((), ()))
MIDSTART = 2

@jax.jit
def pallas_standalone__gqa_block_cached__near_ridge_kernel(x, k_cache, v_cache, wq, wo):
    B, Sq, D = x.shape
    _, Hkv, Sk, Dh = k_cache.shape
    HD = wq.shape[1]
    Hq = HD // Dh
    rep = Hq // Hkv
    GW = rep * Dh
    c = LOG2E * (Dh ** -0.5)
    x2 = x.reshape(B * Sq, D)
    woT = wo.T
    GS = GB // NB
    M = NB * Sq
    nsteps = B // NB
    T = GB * Sq
    XQ = 4
    TH = T // XQ
    NTILE = T // 128
    ngroups = B // GB
    GH = Hkv // QH
    f32, bf16 = jnp.float32, jnp.bfloat16
    S_X0 = 0
    S_X = S_X0 + XQ
    S_WQ = S_X + ngroups
    S_WO = S_WQ + Hkv
    S_KV = S_WO + 1
    S_O = S_KV + NSLOT
    NSEM = S_O + 1

    def kernel(x_hbm, k_hbm, v_hbm, wq_hbm, wo_hbm, o_hbm,
               x_buf, wq_buf, wo_buf, k_buf, v_buf, q_scr, a_scr, o_buf, sems):

        def x0_copy(h):
            return pltpu.make_async_copy(x_hbm.at[pl.ds(h * TH, TH)], x_buf.at[pl.ds(h * TH, TH)],
                                         sems.at[S_X0 + h])

        def x_copy(j):
            return pltpu.make_async_copy(x_hbm.at[pl.ds(j * T, T)], x_buf.at[pl.ds(j * T, T)],
                                         sems.at[S_X + j])

        def wq_copy(g):
            return pltpu.make_async_copy(wq_hbm.at[:, pl.ds(g * GW, GW)],
                                         wq_buf.at[g], sems.at[S_WQ + g])

        def wo_copy():
            return pltpu.make_async_copy(wo_hbm, wo_buf, sems.at[S_WO])

        def kv_copies(step):
            sl = step % NSLOT
            return [
                pltpu.make_async_copy(k_hbm.at[pl.ds(step * NB, NB)], k_buf.at[sl], sems.at[S_KV + sl]),
                pltpu.make_async_copy(v_hbm.at[pl.ds(step * NB, NB)], v_buf.at[sl], sems.at[S_KV + sl]),
            ]

        def o_copy(j, n):
            return pltpu.make_async_copy(o_buf.at[n],
                                         o_hbm.at[pl.ds(j * T + n * 128, 128)], sems.at[S_O])

        x0_copy(0).start()
        wq_copy(0).start()
        for h in range(1, XQ):
            x0_copy(h).start()
        for g in range(1, Hkv):
            wq_copy(g).start()
        for j in range(1, ngroups):
            x_copy(j).start()
        for st in range(NSLOT):
            if st == 2:
                wo_copy().start()
            for cp in kv_copies(st):
                cp.start()

        wq_copy(0).wait()

        def qfirst_rows(h, carry):
            x0_copy(h).wait()
            row = pl.multiple_of(h * TH, 16)
            q = jnp.dot(x_buf[pl.ds(row, TH), :], wq_buf[0], preferred_element_type=f32)
            q_scr[0, 0, pl.ds(row, TH), :] = q.astype(bf16)
            return carry
        lax.fori_loop(0, XQ, qfirst_rows, 0)

        def qfirst_cols(g, carry):
            wq_copy(g).wait()
            q = jnp.dot(x_buf[0:T, :], wq_buf[g], preferred_element_type=f32)
            q_scr[0, g] = q.astype(bf16)
            return carry
        lax.fori_loop(1, GH, qfirst_cols, 0)
        for g in range(GH, Hkv):
            wq_copy(g).wait()

        def qhalf(t, carry):
            j = t // QH
            g0 = (t % QH) * GH
            xb = x_buf[pl.ds(pl.multiple_of(j * T, 16), T), :]
            for gg in range(GH):
                q = jnp.dot(xb, wq_buf[g0 + gg], preferred_element_type=f32)
                q_scr[j % 2, g0 + gg] = q.astype(bf16)
            return carry

        def step(i, carry):
            slot = i % NSLOT
            j = i // GS

            @pl.when(jnp.logical_and(i % GS == 0, j + 1 < ngroups))
            def _():
                x_copy(j + 1).wait()
                lo = jnp.where(i == 0, QH - 1, (j + 1) * QH)
                lax.fori_loop(lo, (j + 2) * QH, qhalf, 0)

            rloc = pl.multiple_of((i % GS) * M, 16)

            def qk(b, g):
                qs = jnp.concatenate(
                    [q_scr[j % 2, g, pl.ds(rloc + b * Sq, Sq), jj * Dh:(jj + 1) * Dh] for jj in range(rep)], axis=0)
                return lax.dot_general(qs, k_buf[slot, b, g], NT, preferred_element_type=f32)

            def pv(b, g, s):
                c0 = g * GW
                m = jnp.max(s, axis=-1, keepdims=True)
                p = jnp.exp2((s - m) * c)
                l = jnp.sum(p, axis=-1, keepdims=True)
                p = p * (1.0 / l)
                o = jnp.dot(p.astype(bf16), v_buf[slot, b, g], preferred_element_type=f32).astype(bf16)
                for jj in range(rep):
                    a_scr[pl.ds(rloc + b * Sq, Sq), c0 + jj * Dh:c0 + (jj + 1) * Dh] = o[jj * Sq:(jj + 1) * Sq]

            def issue_next():
                nxt = i + NSLOT - 1

                @pl.when(jnp.logical_and(i > 0, nxt < nsteps))
                def _():
                    for cp in kv_copies(nxt):
                        cp.start()

            items = [(b, g) for g in range(Hkv) for b in range(NB)]
            for cp in kv_copies(i):
                cp.wait()
            s = qk(*items[0])
            for n, it in enumerate(items):
                s_next = qk(*items[n + 1]) if n + 1 < len(items) else None
                pv(*it, s)
                s = s_next
                if n == MIDSTART:
                    issue_next()

            @pl.when(i % GS == GS - 1)
            def _():
                @pl.when(j == 0)
                def _():
                    wo_copy().wait()

                @pl.when(j > 0)
                def _():
                    for n in range(NTILE):
                        o_copy(j - 1, n).wait()

                for n in range(NTILE):
                    r = lax.dot_general(wo_buf[...], a_scr[n * 128:(n + 1) * 128, :], NT,
                                        preferred_element_type=f32)
                    o_buf[n] = r.T.astype(bf16)
                    o_copy(j, n).start()
            return carry

        lax.fori_loop(0, nsteps, step, 0)
        for n in range(NTILE):
            o_copy(ngroups - 1, n).wait()

    any_spec = pl.BlockSpec(memory_space=pl.ANY)
    out = pl.pallas_call(
        kernel,
        in_specs=[any_spec] * 5,
        out_specs=any_spec,
        out_shape=jax.ShapeDtypeStruct((B * Sq, D), x.dtype),
        scratch_shapes=[
            pltpu.VMEM((B * Sq, D), bf16),
            pltpu.VMEM((Hkv, D, GW), bf16),
            pltpu.VMEM((D, HD), bf16),
            pltpu.VMEM((NSLOT, NB, Hkv, Sk, Dh), bf16),
            pltpu.VMEM((NSLOT, NB, Hkv, Sk, Dh), bf16),
            pltpu.VMEM((2, Hkv, T, GW), bf16),
            pltpu.VMEM((T, HD), bf16),
            pltpu.VMEM((NTILE, 128, D), bf16),
            pltpu.SemaphoreType.DMA((NSEM,)),
        ],
        compiler_params=pltpu.CompilerParams(
            vmem_limit_bytes=110 * 1024 * 1024, disable_bounds_checks=True,
            disable_semaphore_checks=True),
    )(x2, k_cache, v_cache, wq, woT)
    return out.reshape(B, Sq, D)
```

```python
import functools
import jax
import jax.numpy as jnp
from jax import lax
import jax.experimental.pallas as pl
import jax.experimental.pallas.tpu as pltpu

NB = 4
GB = 8
NSLOT = 3
QH = 2
PIN = 1
LOG2E = 1.4426950408889634
NT = (((1,), (1,)), ((), ()))
MIDSTART = 2

@jax.jit
def pallas_standalone__gqa_block_cached__near_ridge_kernel(x, k_cache, v_cache, wq, wo):
    B, Sq, D = x.shape
    _, Hkv, Sk, Dh = k_cache.shape
    HD = wq.shape[1]
    Hq = HD // Dh
    rep = Hq // Hkv
    GW = rep * Dh
    c = LOG2E * (Dh ** -0.5)
    x2 = x.reshape(B * Sq, D)
    woT = wo.T
    GS = GB // NB
    M = NB * Sq
    nsteps = B // NB
    T = GB * Sq
    XQ = 4
    TH = T // XQ
    NTILE = T // 128
    ngroups = B // GB
    GH = Hkv // QH
    f32, bf16 = jnp.float32, jnp.bfloat16
    S_X0 = 0
    S_X = S_X0 + XQ
    S_WQ = S_X + ngroups
    S_WO = S_WQ + Hkv
    S_KV = S_WO + 1
    S_O = S_KV + NSLOT
    NSEM = S_O + 1

    def kernel(x_hbm, k_hbm, v_hbm, wq_hbm, wo_hbm, o_hbm,
               x_buf, wq_buf, wo_buf, k_buf, v_buf, q_scr, a_scr, o_buf, zero_ref, sems):

        def x0_copy(h):
            return pltpu.make_async_copy(x_hbm.at[pl.ds(h * TH, TH)], x_buf.at[pl.ds(h * TH, TH)],
                                         sems.at[S_X0 + h])

        def x_copy(j):
            return pltpu.make_async_copy(x_hbm.at[pl.ds(j * T, T)], x_buf.at[pl.ds(j * T, T)],
                                         sems.at[S_X + j])

        def wq_copy(g):
            return pltpu.make_async_copy(wq_hbm.at[:, pl.ds(g * GW, GW)],
                                         wq_buf.at[g], sems.at[S_WQ + g])

        def wo_copy():
            return pltpu.make_async_copy(wo_hbm, wo_buf, sems.at[S_WO])

        def kv_copies(step):
            sl = step % NSLOT
            return [
                pltpu.make_async_copy(k_hbm.at[pl.ds(step * NB, NB)], k_buf.at[sl], sems.at[S_KV + sl]),
                pltpu.make_async_copy(v_hbm.at[pl.ds(step * NB, NB)], v_buf.at[sl], sems.at[S_KV + sl]),
            ]

        def o_copy(j, n):
            return pltpu.make_async_copy(o_buf.at[(n + j) % NTILE],
                                         o_hbm.at[pl.ds(j * T + n * 128, 128)], sems.at[S_O])

        zero_ref[0] = 0
        x0_copy(0).start()
        wq_copy(0).start()
        for h in range(1, XQ):
            x0_copy(h).start()
        for g in range(1, Hkv):
            wq_copy(g).start()
        for j in range(1, ngroups):
            x_copy(j).start()
        for st in range(NSLOT):
            if st == 2:
                wo_copy().start()
            for cp in kv_copies(st):
                cp.start()

        wq_copy(0).wait()

        def qfirst_rows(h, carry):
            x0_copy(h).wait()
            row = pl.multiple_of(h * TH, 16)
            q = jnp.dot(x_buf[pl.ds(row, TH), :], wq_buf[0], preferred_element_type=f32)
            q_scr[0, 0, pl.ds(row, TH), :] = q.astype(bf16)
            return carry
        lax.fori_loop(0, XQ, qfirst_rows, 0)

        def qfirst_cols(g, carry):
            wq_copy(g).wait()
            q = jnp.dot(x_buf[0:T, :], wq_buf[g], preferred_element_type=f32)
            q_scr[0, g] = q.astype(bf16)
            return carry
        lax.fori_loop(1, GH, qfirst_cols, 0)
        for g in range(GH, Hkv):
            wq_copy(g).wait()

        def qhalf(t, carry):
            j = t // QH
            g0 = (t % QH) * GH
            xb = x_buf[pl.ds(pl.multiple_of(j * T, 16), T), :]
            for gg in range(GH):
                q = jnp.dot(xb, wq_buf[g0 + gg], preferred_element_type=f32)
                q_scr[j % 2, g0 + gg] = q.astype(bf16)
            return carry

        def step(i, carry):
            slot = i % NSLOT
            j = i // GS

            @pl.when(jnp.logical_and(i % GS == 0, j + 1 < ngroups))
            def _():
                x_copy(j + 1).wait()
                lo = jnp.where(i == 0, QH - 1, (j + 1) * QH)
                lax.fori_loop(lo, (j + 2) * QH, qhalf, 0)

            rloc = pl.multiple_of((i % GS) * M, 16)

            def qk(b, g):
                qs = jnp.concatenate(
                    [q_scr[j % 2, g, pl.ds(rloc + b * Sq, Sq), jj * Dh:(jj + 1) * Dh] for jj in range(rep)], axis=0)
                return lax.dot_general(qs, k_buf[slot, b, g], NT, preferred_element_type=f32)

            def pv(b, g, s):
                c0 = g * GW
                m = jnp.max(s, axis=-1, keepdims=True)
                p = jnp.exp2((s - m) * c)
                l = jnp.sum(p, axis=-1, keepdims=True)
                p = p * (1.0 / l)
                o = jnp.dot(p.astype(bf16), v_buf[slot, b, g], preferred_element_type=f32).astype(bf16)
                for jj in range(rep):
                    a_scr[pl.ds(rloc + b * Sq, Sq), c0 + jj * Dh:c0 + (jj + 1) * Dh] = o[jj * Sq:(jj + 1) * Sq]

            def issue_next():
                nxt = i + NSLOT - 1

                @pl.when(jnp.logical_and(i > 0, nxt < nsteps))
                def _():
                    for cp in kv_copies(nxt):
                        cp.start()

            items = [(b, g) for g in range(Hkv) for b in range(NB)]
            for cp in kv_copies(i):
                cp.wait()
            s = qk(*items[0])
            for n, it in enumerate(items):
                s_next = qk(*items[n + 1]) if n + 1 < len(items) else None
                pv(*it, s)
                s = s_next
                if n == MIDSTART:
                    issue_next()

            @pl.when(i % GS == GS - 1)
            def _():
                @pl.when(j == 0)
                def _():
                    wo_copy().wait()

                @pl.when(j > 0)
                def _():
                    for n in range(NTILE):
                        o_copy(j - 1, n).wait()

                z = zero_ref[0].astype(jnp.uint32)
                deps = {}
                for n in range(NTILE):
                    a = a_scr[n * 128:(n + 1) * 128, :]
                    if n in deps:
                        tail = pltpu.bitcast(pltpu.bitcast(a[0:16, HD - 128:], jnp.uint32) | deps[n], bf16)
                        a = jnp.concatenate(
                            [jnp.concatenate([a[0:16, :HD - 128], tail], axis=1), a[16:]], axis=0)
                    r = lax.dot_general(wo_buf[...], a, NT, preferred_element_type=f32)
                    o_buf[(n + j) % NTILE] = r.T.astype(bf16)
                    o_copy(j, n).start()
                    if n + PIN < NTILE:
                        u = pltpu.bitcast(o_buf[(n + j) % NTILE], jnp.uint32)
                        u = functools.reduce(jnp.bitwise_or, [u[8 * k:8 * k + 8] for k in range(8)])
                        nfull = D // 128
                        parts = [u[:, k * 128:(k + 1) * 128] for k in range(nfull)]
                        if D % 128:
                            parts.append(jnp.concatenate(
                                [u[:, nfull * 128:], jnp.zeros((8, 128 - D % 128), jnp.uint32)], axis=1))
                        deps[n + PIN] = functools.reduce(jnp.bitwise_or, parts) & z
            return carry

        lax.fori_loop(0, nsteps, step, 0)
        for n in range(NTILE):
            o_copy(ngroups - 1, n).wait()

    any_spec = pl.BlockSpec(memory_space=pl.ANY)
    out = pl.pallas_call(
        kernel,
        in_specs=[any_spec] * 5,
        out_specs=any_spec,
        out_shape=jax.ShapeDtypeStruct((B * Sq, D), x.dtype),
        scratch_shapes=[
            pltpu.VMEM((B * Sq, D), bf16),
            pltpu.VMEM((Hkv, D, GW), bf16),
            pltpu.VMEM((D, HD), bf16),
            pltpu.VMEM((NSLOT, NB, Hkv, Sk, Dh), bf16),
            pltpu.VMEM((NSLOT, NB, Hkv, Sk, Dh), bf16),
            pltpu.VMEM((2, Hkv, T, GW), bf16),
            pltpu.VMEM((T, HD), bf16),
            pltpu.VMEM((NTILE, 128, D), bf16),
            pltpu.SMEM((1,), jnp.int32),
            pltpu.SemaphoreType.DMA((NSEM,)),
        ],
        compiler_params=pltpu.CompilerParams(
            vmem_limit_bytes=110 * 1024 * 1024, disable_bounds_checks=True,
            disable_semaphore_checks=True),
    )(x2, k_cache, v_cache, wq, woT)
    return out.reshape(B, Sq, D)
```

```python
import functools

import jax
import jax.numpy as jnp
from jax import lax
import jax.experimental.pallas as pl
import jax.experimental.pallas.tpu as pltpu

NB = 4
GB = 8
NSLOT = 3
QH = 2
XQ = 4
MIDSTART = 2
LOG2E = 1.4426950408889634
NT = (((1,), (1,)), ((), ()))


@jax.jit
def pallas_standalone__gqa_block_cached__near_ridge_kernel(x, k_cache, v_cache, wq, wo):
    B, Sq, D = x.shape
    _, Hkv, Sk, Dh = k_cache.shape
    HD = wq.shape[1]
    rep = HD // Dh // Hkv
    GW = rep * Dh
    c = LOG2E * (Dh ** -0.5)
    GS = GB // NB
    M = NB * Sq
    nsteps = B // NB
    T = GB * Sq
    TH = T // XQ
    NTILE = T // 128
    ngroups = B // GB
    GH = Hkv // QH
    f32, bf16, u32 = jnp.float32, jnp.bfloat16, jnp.uint32
    S_X0 = 0
    S_X = S_X0 + XQ
    S_WQ = S_X + ngroups
    S_WO = S_WQ + Hkv
    S_KV = S_WO + 1
    S_O = S_KV + NSLOT
    NSEM = S_O + 1

    def kernel(x_hbm, k_hbm, v_hbm, wq_hbm, wo_hbm, o_hbm,
               x_buf, wq_buf, wo_buf, k_buf, v_buf, q_scr, a_scr, o_buf, zero_ref, sems):

        def x0_copy(h):
            return pltpu.make_async_copy(x_hbm.at[pl.ds(h * TH, TH)], x_buf.at[pl.ds(h * TH, TH)],
                                         sems.at[S_X0 + h])

        def x_copy(j):
            return pltpu.make_async_copy(x_hbm.at[pl.ds(j * T, T)], x_buf.at[pl.ds(j * T, T)],
                                         sems.at[S_X + j])

        def wq_copy(g):
            return pltpu.make_async_copy(wq_hbm.at[:, pl.ds(g * GW, GW)], wq_buf.at[g],
                                         sems.at[S_WQ + g])

        def wo_copy():
            return pltpu.make_async_copy(wo_hbm, wo_buf, sems.at[S_WO])

        def kv_copies(step):
            sl = step % NSLOT
            return [
                pltpu.make_async_copy(k_hbm.at[pl.ds(step * NB, NB)], k_buf.at[sl], sems.at[S_KV + sl]),
                pltpu.make_async_copy(v_hbm.at[pl.ds(step * NB, NB)], v_buf.at[sl], sems.at[S_KV + sl]),
            ]

        def o_copy(j, n):
            return pltpu.make_async_copy(o_buf.at[(n + j) % NTILE],
                                         o_hbm.at[pl.ds(j * T + n * 128, 128)], sems.at[S_O])

        zero_ref[0] = 0

        x0_copy(0).start()
        wq_copy(0).start()
        for h in range(1, XQ):
            x0_copy(h).start()
        for g in range(1, Hkv):
            wq_copy(g).start()
        for j in range(1, ngroups):
            x_copy(j).start()
        for st in range(NSLOT):
            if st == 2:
                wo_copy().start()
            for cp in kv_copies(st):
                cp.start()

        wq_copy(0).wait()

        def qfirst_rows(h, carry):
            x0_copy(h).wait()
            row = pl.multiple_of(h * TH, 16)
            q = jnp.dot(x_buf[pl.ds(row, TH), :], wq_buf[0], preferred_element_type=f32)
            q_scr[0, 0, pl.ds(row, TH), :] = q.astype(bf16)
            return carry
        lax.fori_loop(0, XQ, qfirst_rows, 0)

        def qfirst_cols(g, carry):
            wq_copy(g).wait()
            q = jnp.dot(x_buf[0:T, :], wq_buf[g], preferred_element_type=f32)
            q_scr[0, g] = q.astype(bf16)
            return carry
        lax.fori_loop(1, GH, qfirst_cols, 0)
        for g in range(GH, Hkv):
            wq_copy(g).wait()

        def qblock(t, carry):
            j = t // QH
            g0 = (t % QH) * GH
            xb = x_buf[pl.ds(pl.multiple_of(j * T, 16), T), :]
            for gg in range(GH):
                q = jnp.dot(xb, wq_buf[g0 + gg], preferred_element_type=f32)
                q_scr[j % 2, g0 + gg] = q.astype(bf16)
            return carry

        def step(i, carry):
            slot = i % NSLOT
            j = i // GS

            @pl.when(jnp.logical_and(i % GS == 0, j + 1 < ngroups))
            def _():
                x_copy(j + 1).wait()
                lo = jnp.where(i == 0, 1, (j + 1) * QH)
                lax.fori_loop(lo, (j + 2) * QH, qblock, 0)

            rloc = pl.multiple_of((i % GS) * M, 16)

            def qk(b, g):
                qs = jnp.concatenate(
                    [q_scr[j % 2, g, pl.ds(rloc + b * Sq, Sq), r * Dh:(r + 1) * Dh] for r in range(rep)],
                    axis=0)
                return lax.dot_general(qs, k_buf[slot, b, g], NT, preferred_element_type=f32)

            def softmax_pv(b, g, s):
                m = jnp.max(s, axis=-1, keepdims=True)
                p = jnp.exp2((s - m) * c)
                l = jnp.sum(p, axis=-1, keepdims=True)
                r0 = pl.reciprocal(l, approx=True)
                p = p * (r0 * (2.0 - l * r0))
                o = jnp.dot(p.astype(bf16), v_buf[slot, b, g], preferred_element_type=f32).astype(bf16)
                for r in range(rep):
                    c0 = g * GW + r * Dh
                    a_scr[pl.ds(rloc + b * Sq, Sq), c0:c0 + Dh] = o[r * Sq:(r + 1) * Sq]

            items = [(b, g) for g in range(Hkv) for b in range(NB)]
            for cp in kv_copies(i):
                cp.wait()
            s = qk(*items[0])
            for n, item in enumerate(items):
                s_next = qk(*items[n + 1]) if n + 1 < len(items) else None
                softmax_pv(*item, s)
                s = s_next
                if n == MIDSTART:
                    @pl.when(jnp.logical_and(i > 0, i + NSLOT - 1 < nsteps))
                    def _():
                        for cp in kv_copies(i + NSLOT - 1):
                            cp.start()

            @pl.when(i % GS == GS - 1)
            def _():
                @pl.when(j == 0)
                def _():
                    wo_copy().wait()

                @pl.when(j > 0)
                def _():
                    for n in range(NTILE):
                        o_copy(j - 1, n).wait()

                zero = zero_ref[0].astype(u32)
                dep = None
                for n in range(NTILE):
                    a = a_scr[n * 128:(n + 1) * 128, :]
                    if dep is not None:
                        tail = pltpu.bitcast(pltpu.bitcast(a[0:16, HD - 128:], u32) | dep, bf16)
                        a = jnp.concatenate(
                            [jnp.concatenate([a[0:16, :HD - 128], tail], axis=1), a[16:]], axis=0)
                    r = lax.dot_general(wo_buf[...], a, NT, preferred_element_type=f32)
                    o_buf[(n + j) % NTILE] = r.T.astype(bf16)
                    o_copy(j, n).start()
                    if n + 1 < NTILE:
                        u = pltpu.bitcast(o_buf[(n + j) % NTILE], u32)
                        u = functools.reduce(jnp.bitwise_or, [u[8 * k:8 * k + 8] for k in range(8)])
                        nfull = D // 128
                        parts = [u[:, k * 128:(k + 1) * 128] for k in range(nfull)]
                        if D % 128:
                            parts.append(jnp.concatenate(
                                [u[:, nfull * 128:], jnp.zeros((8, 128 - D % 128), u32)], axis=1))
                        dep = functools.reduce(jnp.bitwise_or, parts) & zero
            return carry

        lax.fori_loop(0, nsteps, step, 0)
        for n in range(NTILE):
            o_copy(ngroups - 1, n).wait()

    any_spec = pl.BlockSpec(memory_space=pl.ANY)
    out = pl.pallas_call(
        kernel,
        in_specs=[any_spec] * 5,
        out_specs=any_spec,
        out_shape=jax.ShapeDtypeStruct((B * Sq, D), x.dtype),
        scratch_shapes=[
            pltpu.VMEM((B * Sq, D), bf16),
            pltpu.VMEM((Hkv, D, GW), bf16),
            pltpu.VMEM((D, HD), bf16),
            pltpu.VMEM((NSLOT, NB, Hkv, Sk, Dh), bf16),
            pltpu.VMEM((NSLOT, NB, Hkv, Sk, Dh), bf16),
            pltpu.VMEM((2, Hkv, T, GW), bf16),
            pltpu.VMEM((T, HD), bf16),
            pltpu.VMEM((NTILE, 128, D), bf16),
            pltpu.SMEM((1,), jnp.int32),
            pltpu.SemaphoreType.DMA((NSEM,)),
        ],
        compiler_params=pltpu.CompilerParams(
            vmem_limit_bytes=110 * 1024 * 1024, disable_bounds_checks=True,
            disable_semaphore_checks=True),
    )(x.reshape(B * Sq, D), k_cache, v_cache, wq, wo.T)
    return out.reshape(B, Sq, D)
```
